```python
import os as _os
_os.environ.setdefault("JAX_PLATFORMS", "cpu")
import jax
import jax.numpy as jnp

def _softmax(x, axis=-1):
    return jax.nn.softmax(x, axis=axis)
def _gelu(x):
    return jax.nn.gelu(x, approximate=True)
def _silu(x):
    return jax.nn.silu(x)
def _sigmoid(x):
    return jax.nn.sigmoid(x)
def _layernorm(x, axis=-1, eps=1e-5):
    m = jnp.mean(x, axis=axis, keepdims=True)
    v = jnp.var(x, axis=axis, keepdims=True)
    return (x - m) / jnp.sqrt(v + eps)
def _scatter_add(tgt, idx, src, axis=0):
    return tgt.at[idx].add(src)
def _segment_sum(src, seg, n):
    return jax.ops.segment_sum(src, seg, n)
class _Rng:
    def __init__(self, key):
        self._k = key
    def _next(self):
        self._k, sub = jax.random.split(self._k)
        return sub
    def normal(self, shape):
        return jax.random.normal(self._next(), shape, dtype=jnp.bfloat16)
    def randint(self, lo, hi, shape):
        return jax.random.randint(self._next(), shape, lo, hi, dtype=jnp.int32)
    def uniform(self, shape, lo=0.0, hi=1.0):
        return jax.random.uniform(self._next(), shape, jnp.bfloat16, lo, hi)
    def permutation(self, n):
        return jax.random.permutation(self._next(), n)


kernel_name = 'interleave_layers__gqa_block_cached__dense_activation_silu__decode'

def setup_inputs():
    _rng = _Rng(jax.random.key(int.from_bytes(__import__("os").urandom(4), "little")))
    _w = (lambda a: (lambda t: t.astype(jnp.bfloat16) if jnp.issubdtype(t.dtype, jnp.floating) else t)(jnp.asarray(a)))
    def _A_setup():
        B, Sq, D = 2, 1, 512
        Hq, Hkv, Sk, Dh = 32, 8, 8192, 128
        assert Hq % Hkv == 0, (Hq, Hkv)
        return {
            "x": _w((lambda *s: _rng.normal(s) * 0.1)(B, Sq, D)),
            "k_cache": _w((lambda *s: _rng.normal(s) * 0.8)(B, Hkv, Sk, Dh)),
            "v_cache": _w((lambda *s: _rng.normal(s) * 1.6)(B, Hkv, Sk, Dh)),
            "wq": _w((lambda *s: _rng.normal(s) * 0.8)(D, Hq * Dh) * (D ** -0.5)),
            "wo": _w((lambda *s: _rng.normal(s) * 1.6)(Hq * Dh, D) * ((Hq * Dh) ** -0.5)),
        }
    _A_in = _A_setup()

    def _B_setup():
        B, S, D, F = 2, 1, 512, 1792
        return {
            "x": _w((lambda *s: _rng.normal(s) * 0.1)(B, S, D)),
            "w1": _w((lambda *s: _rng.normal(s) * 0.4)(D, F) * (D ** -0.5)),
            "w2": _w((lambda *s: _rng.normal(s) * 0.4)(F, D) * (F ** -0.5)),
        }
    _B_in = _B_setup()

    return {
        "A_x": _A_in["x"],
        "A_k_cache": _A_in["k_cache"],
        "A_v_cache": _A_in["v_cache"],
        "A_wq": _A_in["wq"],
        "A_wo": _A_in["wo"],
        "B_x": _B_in["x"],
        "B_w1": _B_in["w1"],
        "B_w2": _B_in["w2"],
    }

def reference(A_x, A_k_cache, A_v_cache, A_wq, A_wo, B_x, B_w1, B_w2):
    def _A_ref(x, k_cache, v_cache, wq, wo):
        B, Sq, D = x.shape
        Hq, Dh = 32, 128
        Hkv = k_cache.shape[1]
        rep = Hq // Hkv
        q = (lambda x, *d: x.transpose(*d))((x @ wq).reshape(B, Sq, Hq, Dh), 0, 2, 1, 3)
        k = jnp.repeat(k_cache, rep, axis=1)
        v = jnp.repeat(v_cache, rep, axis=1)
        scores = jnp.einsum("bhqd,bhkd->bhqk", q, k) * (Dh ** -0.5)
        p = _softmax(scores, axis=-1)
        o = jnp.einsum("bhqk,bhkd->bhqd", p, v)
        return (lambda x, *d: x.transpose(*d))(o, 0, 2, 1, 3).reshape(B, Sq, Hq * Dh) @ wo

    def _B_ref(x, w1, w2):
        h = jnp.einsum("bsd,df->bsf", x, w1)
        h = _silu(h)
        out = jnp.einsum("bsf,fd->bsd", h, w2)
        return out

    x = A_x
    x = x + _A_ref(_layernorm(x, axis=-1), A_k_cache, A_v_cache, A_wq, A_wo)
    x = x + _B_ref(_layernorm(x, axis=-1), B_w1, B_w2)
    x = x + _A_ref(_layernorm(x, axis=-1), A_k_cache, A_v_cache, A_wq, A_wo)
    x = x + _B_ref(_layernorm(x, axis=-1), B_w1, B_w2)
    return x
```

```python
import math

import jax
import jax.numpy as jnp
from jax import lax
import jax.experimental.pallas as pl
import jax.experimental.pallas.tpu as pltpu

_B, _D = 2, 512
_HQ, _HKV, _SK, _DH = 32, 8, 8192, 128
_REP = _HQ // _HKV
_F = 1792
_EPS = 1e-5
_HALF = _SK // 2
_QSCALE = (_DH ** -0.5) * math.log2(math.e)

_NN = (((1,), (0,)), ((), ()))
_NT = (((1,), (1,)), ((), ()))
_F32 = jnp.float32


def _dot(a, b, dims=_NN):
    return lax.dot_general(a, b, dims, preferred_element_type=_F32)


def _rows():
    return lax.broadcasted_iota(jnp.int32, (8, _DH), 0)


def _layernorm(x):
    m = jnp.mean(x, axis=-1, keepdims=True)
    d = x - m
    v = jnp.mean(d * d, axis=-1, keepdims=True)
    return d * lax.rsqrt(v + _EPS)


def _q_pair(xn, wq_ref, h):
    full = _dot(xn, wq_ref[:, pl.ds(h * _REP * _DH, _REP * _DH)]) * _QSCALE
    row = _rows()
    q = full[:, 0:_DH]
    for r in range(1, _REP):
        q = jnp.where(row % _REP == r, full[:, r * _DH:(r + 1) * _DH], q)
    return jnp.where(row < _REP, q, 0.0), jnp.where(row < _REP, 0.0, q)


def _softmax_numer(s):
    m = jnp.max(s, axis=-1, keepdims=True)
    m = jnp.maximum(m, pltpu.roll(m, _REP, 0))
    p = jnp.exp2(s - m)
    l = jnp.sum(p, axis=-1, keepdims=True)
    return p, l + pltpu.roll(l, _REP, 0)


def _merge_halves(acc_a, acc_b, l):
    t = jnp.where(_rows() < _REP, acc_a, acc_b)
    return (t + pltpu.roll(t, _REP, 0)) / l


def _out_proj(o, wo_ref, h):
    row = _rows()
    lhs = jnp.concatenate(
        [jnp.where(row == r, o, 0.0) for r in range(_REP)], axis=1)
    return _dot(lhs, wo_ref[pl.ds(h * _REP * _DH, _REP * _DH), :])


def _sum_rows(a):
    return jnp.broadcast_to(jnp.sum(a, axis=0, keepdims=True), a.shape)


def _ffn(x, w1_ref, w2_ref):
    h = _dot(_layernorm(x), w1_ref[...])
    h = h * jax.nn.sigmoid(h)
    return x + _dot(h, w2_ref[...])


def _kernel(x_hbm, k_hbm, v_hbm, wq_hbm, wo_hbm, w1_hbm, w2_hbm, o_ref,
            x_v, k_v, v_v, kt_v, wq_v, wo_v, w1_v, w2_v, o_v, r_v, sems):
    def copy(src, dst, i):
        return pltpu.make_async_copy(src, dst, sems.at[i])

    cp_x = copy(x_hbm, x_v, 0)
    cp_wq = copy(wq_hbm, wq_v, 1)
    cp_k0 = copy(k_hbm.at[0], k_v.at[0], 2)
    cp_v0 = copy(v_hbm.at[0], v_v.at[0], 3)
    cp_wo = copy(wo_hbm, wo_v, 4)
    cp_w1 = copy(w1_hbm, w1_v, 5)
    cp_w2 = copy(w2_hbm, w2_v, 6)

    def cp_k1(h):
        return copy(k_hbm.at[1, h], k_v.at[1, h], 7 + 2 * h)

    def cp_v1(h):
        return copy(v_hbm.at[1, h], v_v.at[1, h], 8 + 2 * h)

    for c in (cp_x, cp_wq, cp_k0, cp_v0, cp_wo, cp_w1, cp_w2):
        c.start()
    for h in range(_HKV):
        cp_k1(h).start()
        cp_v1(h).start()

    cp_x.wait()
    cp_wq.wait()
    x0 = jnp.broadcast_to(x_v[0:1, :].astype(_F32), (8, _D))
    x1 = jnp.broadcast_to(x_v[1:2, :].astype(_F32), (8, _D))

    def layer_b0(layer, c):
        x = r_v[...]
        xn = _layernorm(x)

        def head(h, carry):
            qa, qb = _q_pair(xn, wq_v, h)

            @pl.when((layer == 0) & (h == 0))
            def _():
                cp_k0.wait()

            s = (_dot(qa, k_v[0, h, 0:_HALF, :], _NT)
                 + _dot(qb, k_v[0, h, _HALF:_SK, :], _NT))
            p, l = _softmax_numer(s)

            @pl.when((layer == 0) & (h == 0))
            def _():
                cp_v0.wait()

            o = _merge_halves(_dot(p, v_v[0, h, 0:_HALF, :]),
                              _dot(p, v_v[0, h, _HALF:_SK, :]), l)
            o_v[h] = o
            return carry

        lax.fori_loop(0, _HKV, head, 0)

        @pl.when(layer == 0)
        def _():
            cp_wo.wait()
            cp_w1.wait()
            cp_w2.wait()

        acc = _out_proj(o_v[0], wo_v, 0)
        for h in range(1, _HKV):
            acc = acc + _out_proj(o_v[h], wo_v, h)
        r_v[...] = _ffn(x + _sum_rows(acc), w1_v, w2_v)
        return c

    r_v[...] = x0
    lax.fori_loop(0, 2, layer_b0, 0)

    xn1 = _layernorm(x1)
    tch = 2048

    def head_b1(h, acc):
        qa, qb = _q_pair(xn1, wq_v, h)
        cp_k1(h).wait()

        def tr(j, c):
            off = pl.multiple_of(j * tch, tch)
            kt_v[h, :, pl.ds(off, tch)] = k_v[1, h, pl.ds(off, tch), :].T
            return c

        lax.fori_loop(0, _SK // tch, tr, 0)
        s = (_dot(qa, kt_v[h, :, 0:_HALF]) + _dot(qb, kt_v[h, :, _HALF:_SK]))
        p, l = _softmax_numer(s)
        cp_v1(h).wait()
        o = _merge_halves(_dot(p, v_v[1, h, 0:_HALF, :]),
                          _dot(p, v_v[1, h, _HALF:_SK, :]), l)
        return acc + _out_proj(o, wo_v, h)

    acc = lax.fori_loop(0, _HKV, head_b1, jnp.zeros((8, _D), _F32))
    x = _ffn(x1 + _sum_rows(acc), w1_v, w2_v)

    xn = _layernorm(x)

    def scores(h):
        qa, qb = _q_pair(xn, wq_v, h)
        return _dot(qa, kt_v[h, :, 0:_HALF]) + _dot(qb, kt_v[h, :, _HALF:_SK])

    s_cur = scores(0)
    acc = None
    o_prev = None
    for h in range(_HKV):
        s_next = scores(h + 1) if h + 1 < _HKV else None
        p, l = _softmax_numer(s_cur)
        o = _merge_halves(_dot(p, v_v[1, h, 0:_HALF, :]),
                          _dot(p, v_v[1, h, _HALF:_SK, :]), l)
        if o_prev is not None:
            t = _out_proj(o_prev, wo_v, h - 1)
            acc = t if acc is None else acc + t
        o_prev, s_cur = o, s_next
    acc = acc + _out_proj(o_prev, wo_v, _HKV - 1)
    y1 = _ffn(x + _sum_rows(acc), w1_v, w2_v)
    row = lax.broadcasted_iota(jnp.int32, (8, _D), 0)
    y = jnp.where(row == 0, r_v[...], y1)
    o_ref[...] = y[0:_B, :].astype(o_ref.dtype)


@jax.jit
def pallas_interleave_layers__gqa_block_cached__dense_activation_silu__decode_kernel(
    A_x: jax.Array,
    A_k_cache: jax.Array,
    A_v_cache: jax.Array,
    A_wq: jax.Array,
    A_wo: jax.Array,
    B_x: jax.Array,
    B_w1: jax.Array,
    B_w2: jax.Array,
):
    del B_x
    bf16 = jnp.bfloat16
    hbm = pl.BlockSpec(memory_space=pl.ANY)
    out = pl.pallas_call(
        _kernel,
        out_shape=jax.ShapeDtypeStruct((_B, _D), A_x.dtype),
        in_specs=[hbm] * 7,
        out_specs=pl.BlockSpec(memory_space=pltpu.VMEM),
        scratch_shapes=[
            pltpu.VMEM((_B, _D), bf16),
            pltpu.VMEM((_B, _HKV, _SK, _DH), bf16),
            pltpu.VMEM((_B, _HKV, _SK, _DH), bf16),
            pltpu.VMEM((_HKV, _DH, _SK), bf16),
            pltpu.VMEM((_D, _HQ * _DH), bf16),
            pltpu.VMEM((_HQ * _DH, _D), bf16),
            pltpu.VMEM((_D, _F), bf16),
            pltpu.VMEM((_F, _D), bf16),
            pltpu.VMEM((_HKV, 8, _DH), _F32),
            pltpu.VMEM((8, _D), _F32),
            pltpu.SemaphoreType.DMA((7 + 2 * _HKV,)),
        ],
        compiler_params=pltpu.CompilerParams(
            vmem_limit_bytes=110 * 1024 * 1024),
        name="gqa_ffn_decode",
    )(A_x.reshape(_B, _D), A_k_cache, A_v_cache, A_wq, A_wo, B_w1, B_w2)
    return out.reshape(_B, 1, _D)
```

```python
import math

import jax
import jax.numpy as jnp
from jax import lax
import jax.experimental.pallas as pl
import jax.experimental.pallas.tpu as pltpu

_B, _D = 2, 512
_HQ, _HKV, _SK, _DH = 32, 8, 8192, 128
_REP = _HQ // _HKV
_G = _REP * _DH
_F = 1792
_EPS = 1e-5
_HALF = _SK // 2
_LAST = _HKV - 1
_QSCALE = (_DH ** -0.5) * math.log2(math.e)
_PIECES = (4096, 2560, 1024, 512)
_NQ_MXU = 2
_SEG = 4

_NN = (((1,), (0,)), ((), ()))
_NT = (((1,), (1,)), ((), ()))
_F32 = jnp.float32
_BF16 = jnp.bfloat16


def _dot(a, b, dims=_NN):
    return lax.dot_general(a, b, dims, preferred_element_type=_F32)


def _rows():
    return lax.broadcasted_iota(jnp.int32, (8, _DH), 0)


def _center(x):
    d = x - jnp.mean(x, axis=-1, keepdims=True)
    return d, lax.rsqrt(jnp.mean(d * d, axis=-1, keepdims=True) + _EPS)


def _split_q(full):
    row = _rows()
    q = full[:, 0:_DH]
    for r in range(1, _REP):
        q = jnp.where(row % _REP == r, full[:, r * _DH:(r + 1) * _DH], q)
    return jnp.where(row < _REP, q, 0.0), jnp.where(row < _REP, 0.0, q)


def _q_pair(d, rstd, wq_ref, h):
    return _split_q(_dot(d, wq_ref[:, pl.ds(h * _G, _G)]) * (rstd * _QSCALE))


def _softmax_numer(s):
    m = jnp.max(s, axis=-1, keepdims=True)
    m = jnp.maximum(m, pltpu.roll(m, _REP, 0))
    p = jnp.exp2(s - m)
    l = jnp.sum(p, axis=-1, keepdims=True)
    return p, l + pltpu.roll(l, _REP, 0)


def _merge_halves(acc_a, acc_b, l):
    t = jnp.where(_rows() < _REP, acc_a, acc_b)
    return (t + pltpu.roll(t, _REP, 0)) / l


def _out_proj(o, wo_ref, h):
    row = _rows()
    lhs = jnp.concatenate(
        [jnp.where(row == r, o, 0.0) for r in range(_REP)], axis=1)
    return _dot(lhs, wo_ref[pl.ds(h * _G, _G), :])


def _sum_rows(a):
    return jnp.broadcast_to(jnp.sum(a, axis=0, keepdims=True), a.shape)


def _ffn(x, w1_ref, w2_ref):
    d, rstd = _center(x)
    h = _dot(d, w1_ref[...]) * rstd
    h = h * jax.nn.sigmoid(h)
    return x + _dot(h, w2_ref[...])


def _column(row):
    return jnp.broadcast_to(row, (_DH, _DH)).T


def _kernel(x_hbm, k_hbm, v_hbm, wq_hbm, wo_hbm, w1_hbm, w2_hbm, o_ref,
            x_v, k_v, v_v, kt_v, wq_v, wo_v, w1_v, w2_v, o_v, r_v,
            wq32, wo32, xc_v, z_v, sems):
    def copy(src, dst, i):
        return pltpu.make_async_copy(src, dst, sems.at[i])

    cp_x = copy(x_hbm, x_v, 0)
    cp_wq = copy(wq_hbm, wq_v, 1)
    cp_k0 = copy(k_hbm.at[0], k_v.at[0], 2)
    cp_v0 = copy(v_hbm.at[0], v_v.at[0], 3)
    cp_wo = copy(wo_hbm, wo_v, 4)
    cp_w1 = copy(w1_hbm, w1_v, 5)
    cp_w2 = copy(w2_hbm, w2_v, 6)

    def cp_k1(h):
        return copy(k_hbm.at[1, h], k_v.at[1, h], 7 + h)

    def cp_v1(h):
        return copy(v_hbm.at[1, h], v_v.at[1, h], 7 + _HKV + h)

    starts = [sum(_PIECES[:i]) for i in range(len(_PIECES))]
    cp_vl = [copy(v_hbm.at[1, _LAST, pl.ds(lo, n)], v_v.at[1, _LAST, pl.ds(lo, n)],
                  7 + _HKV + _LAST + i)
             for i, (lo, n) in enumerate(zip(starts, _PIECES))]

    for c in (cp_x, cp_wq, cp_k0, cp_v0, cp_wo, cp_w1, cp_w2):
        c.start()
    for h in range(_LAST):
        cp_k1(h).start()
        if h == _LAST - 1:
            cp_k1(_LAST).start()
        cp_v1(h).start()
    for c in cp_vl:
        c.start()

    v_u = v_v.bitcast(jnp.uint32)

    def vals(b, h, lo, n):
        return pltpu.bitcast(v_u[b, h, pl.ds(lo // 2, n // 2), :], _BF16)

    z_v[...] = jnp.zeros((8, _DH), jnp.int32)
    cp_x.wait()
    cp_wq.wait()
    x0 = jnp.broadcast_to(x_v[0:1, :].astype(_F32), (8, _D))
    x1 = jnp.broadcast_to(x_v[1:2, :].astype(_F32), (8, _D))

    def layer_b0(layer, c):
        x = r_v[...]
        d, rstd = _center(x)

        def head(h, carry):
            qa, qb = _q_pair(d, rstd, wq_v, h)
            pl.when((layer == 0) & (h == 0))(cp_k0.wait)
            s = (_dot(qa, k_v[0, h, 0:_HALF, :], _NT)
                 + _dot(qb, k_v[0, h, _HALF:_SK, :], _NT))
            p, l = _softmax_numer(s)
            pl.when((layer == 0) & (h == 0))(cp_v0.wait)
            o_v[h] = _merge_halves(_dot(p, vals(0, h, 0, _HALF)),
                                   _dot(p, vals(0, h, _HALF, _HALF)), l)
            return carry

        lax.fori_loop(0, _HKV, head, 0)

        @pl.when(layer == 0)
        def _():
            cp_wo.wait()
            cp_w1.wait()
            cp_w2.wait()

        acc = _out_proj(o_v[0], wo_v, 0)
        for h in range(1, _HKV):
            acc = acc + _out_proj(o_v[h], wo_v, h)
        r_v[...] = _ffn(x + _sum_rows(acc), w1_v, w2_v)
        return c

    r_v[...] = x0
    lax.fori_loop(0, 2, layer_b0, 0)

    d1, rstd1 = _center(x1)

    def transpose_keys(h):
        kt_v[h] = pltpu.bitcast(k_v[1, h].T, jnp.uint32)

    def scores(q, h):
        return (_dot(q[0], pltpu.bitcast(kt_v[h, :, 0:_HALF], _BF16))
                + _dot(q[1], pltpu.bitcast(kt_v[h, :, _HALF:_SK], _BF16)))

    def head_b1(h, acc):
        q = _q_pair(d1, rstd1, wq_v, h)
        off = pl.multiple_of(h * _G, _G)
        wq32[h] = wq_v[:, pl.ds(off + _G, _G)].astype(_F32)
        wo32[h] = wo_v[pl.ds(off, _G), :].astype(_F32)
        cp_k1(h).wait()
        transpose_keys(h)
        p, l = _softmax_numer(scores(q, h))

        @pl.when(h == _LAST - 1)
        def _():
            cp_k1(_LAST).wait()
            transpose_keys(_LAST)

        cp_v1(h).wait()
        o = _merge_halves(_dot(p, vals(1, h, 0, _HALF)),
                          _dot(p, vals(1, h, _HALF, _HALF)), l)
        return acc + _out_proj(o, wo_v, h)

    acc = lax.fori_loop(0, _LAST, head_b1, jnp.zeros((8, _D), _F32))
    p, l = _softmax_numer(scores(_q_pair(d1, rstd1, wq_v, _LAST), _LAST))
    halves = [None, None]
    for lo, n, c in zip(starts, _PIECES, cp_vl):
        c.wait()
        t = _dot(p[:, lo % _HALF:lo % _HALF + n], vals(1, _LAST, lo, n))
        hf = lo // _HALF
        halves[hf] = t if halves[hf] is None else halves[hf] + t
    acc = acc + _out_proj(_merge_halves(halves[0], halves[1], l), wo_v, _LAST)
    x = _ffn(x1 + _sum_rows(acc), w1_v, w2_v)

    d, rstd = _center(x)
    zero = z_v[...]

    def after(*vs):
        t = zero
        for v in vs:
            t = t & pltpu.bitcast(v, jnp.int32)
        return pltpu.bitcast(t, _F32)

    def mac(a, w_ref, slab, k0, c):
        for j in range(len(a)):
            t = w_ref[slab, k0:k0 + 8, j * _DH:(j + 1) * _DH] * c
            a[j] = t if a[j] is None else a[j] + t

    def q_vpu(h, s):
        a = [None] * (_G // _DH)
        ng = _D // 8
        for g in range(ng):
            c = xc_v[8 * g:8 * g + 8, :]
            if g % (ng // _SEG) == 0:
                lo = g * (_HALF // ng)
                c = c + after(s[:, lo:lo + _DH])
            mac(a, wq32, h - 1, 8 * g, c)
        return _split_q(_sum_rows(jnp.concatenate(a, axis=1)) * (rstd * _QSCALE))

    def o_vpu(o, h, a, clocks):
        for r in range(_REP):
            col = _column(o[r:r + 1, :])
            for g in range(_DH // 8):
                c = col[8 * g:8 * g + 8, :]
                if g == 0:
                    c = c + after(clocks[r])
                mac(a, wo32, h, r * _DH + 8 * g, c)

    qs = {h: _q_pair(d, rstd, wq_v, h) for h in range(_NQ_MXU)}
    for j in range(_D // _DH):
        xc_v[j * _DH:(j + 1) * _DH, :] = _column(d[0:1, j * _DH:(j + 1) * _DH])

    a = [None] * (_D // _DH)
    s_cur = scores(qs[0], 0)
    o_prev = None
    for h in range(_HKV):
        s_next = None
        if h + 1 < _HKV:
            qa, qb = qs[h + 1]
            if a[0] is not None:
                qb = qb + after(*a)
            s_next = scores((qa, qb), h + 1)
            if h + 2 < _HKV and h + 2 not in qs:
                qs[h + 2] = q_vpu(h + 2, s_next)
        p, l = _softmax_numer(s_cur)
        n = _SK // 4
        parts = [_dot(p[:, (i * n) % _HALF:(i * n) % _HALF + n], vals(1, h, i * n, n))
                 for i in range(4)]
        if o_prev is not None:
            o_vpu(o_prev, h - 1, a, [p[:, 0:_DH]] * 3 + [parts[0]])
        o_prev = _merge_halves(parts[0] + parts[1], parts[2] + parts[3], l)
        s_cur = s_next
    acc = _out_proj(o_prev, wo_v, _LAST) + jnp.concatenate(a, axis=1)
    y1 = _ffn(x + _sum_rows(acc), w1_v, w2_v)

    row = lax.broadcasted_iota(jnp.int32, (8, _D), 0)
    y = jnp.where(row == 0, r_v[...], y1)
    o_ref[...] = y[0:_B, :].astype(o_ref.dtype)


@jax.jit
def pallas_interleave_layers__gqa_block_cached__dense_activation_silu__decode_kernel(
    A_x: jax.Array,
    A_k_cache: jax.Array,
    A_v_cache: jax.Array,
    A_wq: jax.Array,
    A_wo: jax.Array,
    B_x: jax.Array,
    B_w1: jax.Array,
    B_w2: jax.Array,
):
    del B_x
    hbm = pl.BlockSpec(memory_space=pl.ANY)
    out = pl.pallas_call(
        _kernel,
        out_shape=jax.ShapeDtypeStruct((_B, _D), A_x.dtype),
        in_specs=[hbm] * 7,
        out_specs=pl.BlockSpec(memory_space=pltpu.VMEM),
        scratch_shapes=[
            pltpu.VMEM((_B, _D), _BF16),
            pltpu.VMEM((_B, _HKV, _SK, _DH), _BF16),
            pltpu.VMEM((_B, _HKV, _SK, _DH), _BF16),
            pltpu.VMEM((_HKV, _DH // 2, _SK), jnp.uint32),
            pltpu.VMEM((_D, _HQ * _DH), _BF16),
            pltpu.VMEM((_HQ * _DH, _D), _BF16),
            pltpu.VMEM((_D, _F), _BF16),
            pltpu.VMEM((_F, _D), _BF16),
            pltpu.VMEM((_HKV, 8, _DH), _F32),
            pltpu.VMEM((8, _D), _F32),
            pltpu.VMEM((_LAST, _D, _G), _F32),
            pltpu.VMEM((_LAST, _G, _D), _F32),
            pltpu.VMEM((_D, _DH), _F32),
            pltpu.VMEM((8, _DH), jnp.int32),
            pltpu.SemaphoreType.DMA((7 + _HKV + _LAST + len(_PIECES),)),
        ],
        compiler_params=pltpu.CompilerParams(
            vmem_limit_bytes=120 * 1024 * 1024),
        name="gqa_ffn_decode",
    )(A_x.reshape(_B, _D), A_k_cache, A_v_cache, A_wq, A_wo, B_w1, B_w2)
    return out.reshape(_B, 1, _D)
```
